```python
import jax
import jax.numpy as jnp

def _softmax(x, axis=-1):
    return jax.nn.softmax(x, axis=axis)

def _gelu(x):
    return jax.nn.gelu(x, approximate=True)

def _silu(x):
    return jax.nn.silu(x)

def _sigmoid(x):
    return jax.nn.sigmoid(x)

def _layernorm(x, axis=-1, eps=1e-05):
    m = jnp.mean(x, axis=axis, keepdims=True)
    v = jnp.var(x, axis=axis, keepdims=True)
    return (x - m) / jnp.sqrt(v + eps)

def _scatter_add(tgt, idx, src, axis=0):
    return tgt.at[idx].add(src)

def _segment_sum(src, seg, n):
    return jax.ops.segment_sum(src, seg, n)

class _Rng:

    def __init__(self, key):
        self._k = key

    def _next(self):
        self._k, sub = jax.random.split(self._k)
        return sub

    def normal(self, shape):
        return jax.random.normal(self._next(), shape, dtype=jnp.bfloat16)

    def randint(self, lo, hi, shape):
        return jax.random.randint(self._next(), shape, lo, hi, dtype=jnp.int32)

    def uniform(self, shape, lo=0.0, hi=1.0):
        return jax.random.uniform(self._next(), shape, jnp.bfloat16, lo, hi)

    def permutation(self, n):
        return jax.random.permutation(self._next(), n)
kernel_name = 'adaLN_cond__sliding_block_cached__mixer_gmlp__decode'

def setup_inputs():
    _rng = _Rng(jax.random.key(int.from_bytes(__import__("os").urandom(4), "little")))
    _w = lambda a: (lambda t: t.astype(jnp.bfloat16) if jnp.issubdtype(t.dtype, jnp.floating) else t)(jnp.asarray(a))

    def _A_setup():
        B, Sq, D = (1, 1, 448)
        Hq, Hkv, Sk, Dh = (16, 8, 65536, 256)
        assert Hq % Hkv == 0, (Hq, Hkv)
        return {'x': _w((lambda *s: _rng.normal(s) * 0.05)(B, Sq, D)), 'k_cache': _w((lambda *s: _rng.normal(s) * 0.05)(B, Hkv, Sk, Dh)), 'v_cache': _w((lambda *s: _rng.normal(s) * 0.05)(B, Hkv, Sk, Dh)), 'wq': _w((lambda *s: _rng.normal(s) * 0.05)(D, Hq * Dh) * D ** (-0.5)), 'wo': _w((lambda *s: _rng.normal(s) * 0.05)(Hq * Dh, D) * (Hq * Dh) ** (-0.5))}
    _A_in = _A_setup()

    def _B_setup():
        B, S, D, F = (1, 1, 448, 1792)
        Fh = F // 2
        return {'x': _w((lambda *s: _rng.normal(s) * 0.05)(B, S, D)), 'w_in': _w((lambda *s: _rng.normal(s) * 0.05)(D, 2 * Fh)), 'w_sp': _w(0.01 * (lambda *s: _rng.normal(s) * 0.05)(S, S)), 'b_sp': _w(1.0 + 0.01 * (lambda *s: _rng.normal(s) * 0.05)(S)), 'w_out': _w((lambda *s: _rng.normal(s) * 0.05)(Fh, D))}
    _B_in = _B_setup()
    return {'A_x': _A_in['x'], 'A_k_cache': _A_in['k_cache'], 'A_v_cache': _A_in['v_cache'], 'A_wq': _A_in['wq'], 'A_wo': _A_in['wo'], 'B_x': _B_in['x'], 'B_w_in': _B_in['w_in'], 'B_w_sp': _B_in['w_sp'], 'B_b_sp': _B_in['b_sp'], 'B_w_out': _B_in['w_out'], 'c': _w((lambda *s: _rng.normal(s) * 0.05)(1, 448)), 'w_mod': _w((lambda *s: _rng.normal(s) * 0.05)(448, 6 * 448) * 448 ** (-0.5))}

def reference(A_x, A_k_cache, A_v_cache, A_wq, A_wo, B_x, B_w_in, B_w_sp, B_b_sp, B_w_out, c, w_mod):

    def _A_ref(x, k_cache, v_cache, wq, wo):
        B, Sq, D = x.shape
        Hq, Dh = (16, 256)
        Hkv, Sk = (k_cache.shape[1], k_cache.shape[2])
        W = min(4096, max(256, Sk // 4))
        rep = Hq // Hkv
        q = (lambda x, *d: x.transpose(*d))((x @ wq).reshape(B, Sq, Hq, Dh), 0, 2, 1, 3)
        k = jnp.repeat(k_cache[:, :, Sk - W:, :], rep, axis=1)
        v = jnp.repeat(v_cache[:, :, Sk - W:, :], rep, axis=1)
        scores = jnp.einsum('bhqd,bhkd->bhqk', q, k) * Dh ** (-0.5)
        p = _softmax(scores, axis=-1)
        o = jnp.einsum('bhqk,bhkd->bhqd', p, v)
        return (lambda x, *d: x.transpose(*d))(o, 0, 2, 1, 3).reshape(B, Sq, Hq * Dh) @ wo

    def _B_ref(x, w_in, w_sp, b_sp, w_out):
        B, S, D = x.shape
        F = w_in.shape[-1]
        Fh = F // 2
        z = _gelu(jnp.einsum('bsd,df->bsf', x, w_in))
        z1 = z[..., :Fh].copy()
        z2 = _layernorm(z[..., Fh:], axis=-1)
        g = jnp.einsum('ts,bsf->btf', w_sp, z2) + b_sp[None, :, None]
        return jnp.einsum('bsf,fd->bsd', z1 * g, w_out)
    x = A_x
    mod = (_silu(c) @ w_mod).reshape(c.shape[0], 6, 1, -1)
    sa, ca, ga, sb, cb, gb = (mod[:, 0].copy(), mod[:, 1].copy(), mod[:, 2].copy(), mod[:, 3].copy(), mod[:, 4].copy(), mod[:, 5].copy())
    h = _layernorm(x, axis=-1) * (1 + ca) + sa
    x = x + ga * _A_ref(h, A_k_cache, A_v_cache, A_wq, A_wo)
    h = _layernorm(x, axis=-1) * (1 + cb) + sb
    x = x + gb * _B_ref(h, B_w_in, B_w_sp, B_b_sp, B_w_out)
    return x
```

```python
import functools
import jax
import jax.numpy as jnp
from jax import lax
import jax.experimental.pallas as pl
import jax.experimental.pallas.tpu as pltpu

D = 448
HQ, HKV, DH = 16, 8, 256
F = 1792
FH = F // 2
EPS = 1e-5
WOUT_SPLITS = (0, 640, 896)
DISABLE_SEM_CHECKS = True


def _ln(x):
    m = jnp.mean(x, axis=-1, keepdims=True)
    d = x - m
    v = jnp.mean(d * d, axis=-1, keepdims=True)
    return d / jnp.sqrt(v + EPS)


def _nt(a, b):
    return lax.dot_general(a, b, (((1,), (1,)), ((), ())), preferred_element_type=jnp.float32)


def _nn(a, b):
    return lax.dot_general(a, b, (((1,), (0,)), ((), ())), preferred_element_type=jnp.float32)


def _mod_chunk(mod, i):
    start = i * D
    t0 = (start // 128) * 128
    sh = start - t0
    if sh == 0:
        return mod[:, start:start + D]
    slab = mod[:, t0:t0 + 512]
    return pltpu.roll(slab, 512 - sh, 1)[:, :D]


def _kernel(x_hbm, k_hbm, v_hbm, wq_hbm, woT_hbm, win_hbm, wsp_hbm, bsp_hbm, woutT_hbm, c_hbm, wmod_hbm,
            o_ref,
            x_v, c_v, wsp_v, bsp_v, wmod_v, wq_v, woT_v, win_v, woutT_v, k_v, v_v, sems, *, Sk, W):
    bf = jnp.bfloat16
    f32 = jnp.float32
    copies = {}
    n = [0]

    def mk(name, src, dst):
        cp = pltpu.make_async_copy(src, dst, sems.at[n[0]])
        n[0] += 1
        copies[name] = cp
        cp.start()

    mk('c', c_hbm, c_v)
    mk('x', x_hbm, x_v)
    mk('wmod', wmod_hbm, wmod_v)
    mk('wq', wq_hbm, wq_v)
    mk('k', k_hbm.at[0, :, pl.ds(Sk - W, W), :], k_v)
    mk('v', v_hbm.at[0, :, pl.ds(Sk - W, W), :], v_v)
    mk('wo', woT_hbm, woT_v)
    mk('win', win_hbm, win_v)
    nsp = len(WOUT_SPLITS) - 1
    for j in range(nsp):
        a, b = WOUT_SPLITS[j], WOUT_SPLITS[j + 1]
        mk(f'wout{j}', woutT_hbm.at[:, pl.ds(a, b - a)], woutT_v.at[:, pl.ds(a, b - a)])
    mk('wsp', wsp_hbm, wsp_v)
    mk('bsp', bsp_hbm, bsp_v)

    copies['c'].wait()
    c = c_v[...].astype(f32)
    sc = c * (1.0 / (1.0 + jnp.exp(-c)))
    sc8 = jnp.broadcast_to(sc, (8, D)).astype(bf)
    copies['x'].wait()
    x = jnp.broadcast_to(x_v[0].astype(f32), (8, D))
    xn = _ln(x)
    copies['wmod'].wait()
    mod = _nn(sc8, wmod_v[...])
    sa, ca, ga, sb, cb, gb = [_mod_chunk(mod, i) for i in range(6)]
    h1 = (xn * (1.0 + ca) + sa).astype(bf)
    copies['wq'].wait()
    row = lax.broadcasted_iota(jnp.int32, (8, DH), 0)
    qs = []
    for g in range(2):
        acc = jnp.zeros((8, DH), f32)
        for r in range(8):
            i = g * 8 + r
            qi = _nn(h1, wq_v[:, i * DH:(i + 1) * DH])
            acc = jnp.where(row == r, qi, acc)
        qs.append(acc.astype(bf))
    scale = DH ** -0.5
    rowW = lax.broadcasted_iota(jnp.int32, (8, W), 0)
    copies['k'].wait()
    ps, ls = [], []
    for g in range(2):
        s = jnp.zeros((8, W), f32)
        for j in range(4):
            sh = _nt(qs[g], k_v[4 * g + j])
            s = jnp.where((rowW // 2) == j, sh, s)
        s = s * scale
        m = jnp.max(s, axis=-1, keepdims=True)
        p = jnp.exp(s - m)
        ls.append(jnp.sum(p, axis=-1, keepdims=True))
        ps.append(p.astype(bf))
    copies['v'].wait()
    Os = []
    for g in range(2):
        o = jnp.zeros((8, DH), f32)
        for j in range(4):
            oh = _nn(ps[g], v_v[4 * g + j])
            o = jnp.where((row // 2) == j, oh, o)
        Os.append(o / ls[g])
    copies['wo'].wait()
    att = jnp.zeros((8, D), f32)
    for i in range(HQ):
        lhs = jnp.where(row == (i % 8), Os[i // 8], 0.0).astype(bf)
        att = att + _nt(lhs, woT_v[:, i * DH:(i + 1) * DH])
    att = jnp.broadcast_to(jnp.sum(att, axis=0, keepdims=True), (8, D))
    x2 = x + ga * att
    h2 = (_ln(x2) * (1.0 + cb) + sb).astype(bf)
    copies['win'].wait()
    z = _nn(h2, win_v[...])
    z = jax.nn.gelu(z, approximate=True)
    z1 = z[:, :FH]
    z2 = _ln(z[:, FH:])
    copies['wsp'].wait()
    copies['bsp'].wait()
    wsp = wsp_v[...].astype(f32)
    bsp = bsp_v[...].astype(f32).reshape(1, 1)
    g = wsp * z2 + bsp
    u = (z1 * g).astype(bf)
    base = x2
    for j in range(nsp):
        a, b = WOUT_SPLITS[j], WOUT_SPLITS[j + 1]
        copies[f'wout{j}'].wait()
        y = _nt(u[:, a:b], woutT_v[:, a:b])
        base = base + gb * y
    o_ref[0] = base[0:1].astype(o_ref.dtype)


@jax.jit
def pallas_adaLN_cond__sliding_block_cached__mixer_gmlp__decode_kernel(
    A_x, A_k_cache, A_v_cache, A_wq, A_wo, B_x, B_w_in, B_w_sp, B_b_sp, B_w_out, c, w_mod):
    Sk = A_k_cache.shape[2]
    W = min(4096, max(256, Sk // 4))
    bf = jnp.bfloat16
    any_spec = pl.BlockSpec(memory_space=pltpu.HBM)
    nsem = 10 + len(WOUT_SPLITS) - 1
    scratch = [
        pltpu.VMEM((1, 1, D), bf), pltpu.VMEM((1, D), bf), pltpu.VMEM((1, 1), bf), pltpu.VMEM((1,), bf),
        pltpu.VMEM((D, 6 * D), bf), pltpu.VMEM((D, HQ * DH), bf), pltpu.VMEM((D, HQ * DH), bf),
        pltpu.VMEM((D, F), bf), pltpu.VMEM((D, FH), bf),
        pltpu.VMEM((HKV, W, DH), bf), pltpu.VMEM((HKV, W, DH), bf),
        pltpu.SemaphoreType.DMA((nsem,)),
    ]
    return pl.pallas_call(
        functools.partial(_kernel, Sk=Sk, W=W),
        out_shape=jax.ShapeDtypeStruct(A_x.shape, A_x.dtype),
        in_specs=[any_spec] * 11,
        out_specs=pl.BlockSpec(memory_space=pltpu.VMEM),
        scratch_shapes=scratch,
        compiler_params=pltpu.CompilerParams(vmem_limit_bytes=100 * 1024 * 1024,
                                             disable_semaphore_checks=DISABLE_SEM_CHECKS),
    )(A_x, A_k_cache, A_v_cache, A_wq, A_wo.T, B_w_in, B_w_sp, B_b_sp, B_w_out.T, c, w_mod)
```

```python
import functools

import jax
import jax.numpy as jnp
from jax import lax
import jax.experimental.pallas as pl
import jax.experimental.pallas.tpu as pltpu

_D = 448
_HQ, _HKV, _DH = 16, 8, 256
_F = 1792
_FH = _F // 2
_EPS = 1e-5
_WOUT_SPLITS = (0, 640, _FH)

_F32 = jnp.float32
_BF16 = jnp.bfloat16


def _layernorm(x):
    m = jnp.mean(x, axis=-1, keepdims=True)
    d = x - m
    v = jnp.mean(d * d, axis=-1, keepdims=True)
    return d / jnp.sqrt(v + _EPS)


def _mm_nn(a, b):
    return lax.dot_general(a, b, (((1,), (0,)), ((), ())), preferred_element_type=_F32)


def _mm_nt(a, b):
    return lax.dot_general(a, b, (((1,), (1,)), ((), ())), preferred_element_type=_F32)


def _mod_chunk(mod, i):
    start = i * _D
    tile0 = (start // 128) * 128
    shift = start - tile0
    if shift == 0:
        return mod[:, start:start + _D]
    slab = mod[:, tile0:tile0 + 512]
    return pltpu.roll(slab, 512 - shift, 1)[:, :_D]


def _kernel(x_hbm, k_hbm, v_hbm, wq_hbm, wot_hbm, win_hbm, wsp_hbm, bsp_hbm, woutt_hbm,
            c_hbm, wmod_hbm,
            o_ref,
            x_v, c_v, wsp_v, bsp_v, wmod_v, wq_v, wot_v, win_v, woutt_v, k_v, v_v, sems,
            *, sk, w):
    copies = {}

    def start_copy(name, src, dst):
        cp = pltpu.make_async_copy(src, dst, sems.at[len(copies)])
        cp.start()
        copies[name] = cp

    start_copy("c", c_hbm, c_v)
    start_copy("x", x_hbm, x_v)
    start_copy("wmod", wmod_hbm, wmod_v)
    start_copy("wq", wq_hbm, wq_v)
    start_copy("k", k_hbm.at[0, :, pl.ds(sk - w, w), :], k_v)
    start_copy("v", v_hbm.at[0, :, pl.ds(sk - w, w), :], v_v)
    start_copy("wo", wot_hbm, wot_v)
    start_copy("win", win_hbm, win_v)
    n_wout = len(_WOUT_SPLITS) - 1
    for j in range(n_wout):
        a, b = _WOUT_SPLITS[j], _WOUT_SPLITS[j + 1]
        start_copy(f"wout{j}", woutt_hbm.at[:, pl.ds(a, b - a)], woutt_v.at[:, pl.ds(a, b - a)])
    start_copy("wsp", wsp_hbm, wsp_v)
    start_copy("bsp", bsp_hbm, bsp_v)

    copies["c"].wait()
    c = c_v[...].astype(_F32)
    silu_c = c * (1.0 / (1.0 + jnp.exp(-c)))
    silu_c = jnp.broadcast_to(silu_c, (8, _D)).astype(_BF16)
    copies["x"].wait()
    x = jnp.broadcast_to(x_v[0].astype(_F32), (8, _D))
    xn = _layernorm(x)
    copies["wmod"].wait()
    mod = _mm_nn(silu_c, wmod_v[...])
    sa, ca, ga, sb, cb, gb = [_mod_chunk(mod, i) for i in range(6)]
    h1 = (xn * (1.0 + ca) + sa).astype(_BF16)

    copies["wq"].wait()
    row = lax.broadcasted_iota(jnp.int32, (8, _DH), 0)
    q = []
    for g in range(2):
        acc = jnp.zeros((8, _DH), _F32)
        for r in range(8):
            i = 8 * g + r
            qi = _mm_nn(h1, wq_v[:, i * _DH:(i + 1) * _DH])
            acc = jnp.where(row == r, qi, acc)
        q.append(acc.astype(_BF16))

    copies["k"].wait()
    row_w = lax.broadcasted_iota(jnp.int32, (8, w), 0)
    p, denom = [], []
    for g in range(2):
        s = jnp.zeros((8, w), _F32)
        for j in range(4):
            sj = _mm_nt(q[g], k_v[4 * g + j])
            s = jnp.where((row_w // 2) == j, sj, s)
        s = s * (_DH ** -0.5)
        m = jnp.max(s, axis=-1, keepdims=True)
        e = jnp.exp(s - m)
        denom.append(jnp.sum(e, axis=-1, keepdims=True))
        p.append(e.astype(_BF16))

    copies["v"].wait()
    o = []
    for g in range(2):
        acc = jnp.zeros((8, _DH), _F32)
        for j in range(4):
            oj = _mm_nn(p[g], v_v[4 * g + j])
            acc = jnp.where((row // 2) == j, oj, acc)
        o.append(acc / denom[g])

    copies["wo"].wait()
    att = jnp.zeros((8, _D), _F32)
    for i in range(_HQ):
        oi = jnp.where(row == (i % 8), o[i // 8], 0.0).astype(_BF16)
        att = att + _mm_nt(oi, wot_v[:, i * _DH:(i + 1) * _DH])
    att = jnp.broadcast_to(jnp.sum(att, axis=0, keepdims=True), (8, _D))
    x2 = x + ga * att
    h2 = (_layernorm(x2) * (1.0 + cb) + sb).astype(_BF16)

    copies["win"].wait()
    z = jax.nn.gelu(_mm_nn(h2, win_v[...]), approximate=True)
    z1 = z[:, :_FH]
    z2 = _layernorm(z[:, _FH:])
    copies["wsp"].wait()
    copies["bsp"].wait()
    w_sp = wsp_v[...].astype(_F32)
    b_sp = bsp_v[...].astype(_F32).reshape(1, 1)
    u = (z1 * (w_sp * z2 + b_sp)).astype(_BF16)

    out = x2
    for j in range(n_wout):
        a, b = _WOUT_SPLITS[j], _WOUT_SPLITS[j + 1]
        copies[f"wout{j}"].wait()
        out = out + gb * _mm_nt(u[:, a:b], woutt_v[:, a:b])
    o_ref[0] = out[0:1].astype(o_ref.dtype)


@jax.jit
def pallas_adaLN_cond__sliding_block_cached__mixer_gmlp__decode_kernel(
    A_x: jax.Array,
    A_k_cache: jax.Array,
    A_v_cache: jax.Array,
    A_wq: jax.Array,
    A_wo: jax.Array,
    B_x: jax.Array,
    B_w_in: jax.Array,
    B_w_sp: jax.Array,
    B_b_sp: jax.Array,
    B_w_out: jax.Array,
    c: jax.Array,
    w_mod: jax.Array,
):
    del B_x
    assert A_x.shape == (1, 1, _D) and c.shape == (1, _D)
    assert A_k_cache.shape == A_v_cache.shape
    assert (A_k_cache.shape[0], A_k_cache.shape[1], A_k_cache.shape[3]) == (1, _HKV, _DH)
    assert A_wq.shape == (_D, _HQ * _DH) and A_wo.shape == (_HQ * _DH, _D)
    assert B_w_in.shape == (_D, _F) and B_w_out.shape == (_FH, _D)
    assert B_w_sp.shape == (1, 1) and B_b_sp.shape == (1,) and w_mod.shape == (_D, 6 * _D)
    sk = A_k_cache.shape[2]
    w = min(4096, max(256, sk // 4))

    hbm = pl.BlockSpec(memory_space=pltpu.HBM)
    n_copies = 10 + len(_WOUT_SPLITS) - 1
    scratch_shapes = [
        pltpu.VMEM((1, 1, _D), _BF16),
        pltpu.VMEM((1, _D), _BF16),
        pltpu.VMEM((1, 1), _BF16),
        pltpu.VMEM((1,), _BF16),
        pltpu.VMEM((_D, 6 * _D), _BF16),
        pltpu.VMEM((_D, _HQ * _DH), _BF16),
        pltpu.VMEM((_D, _HQ * _DH), _BF16),
        pltpu.VMEM((_D, _F), _BF16),
        pltpu.VMEM((_D, _FH), _BF16),
        pltpu.VMEM((_HKV, w, _DH), _BF16),
        pltpu.VMEM((_HKV, w, _DH), _BF16),
        pltpu.SemaphoreType.DMA((n_copies,)),
    ]
    return pl.pallas_call(
        functools.partial(_kernel, sk=sk, w=w),
        out_shape=jax.ShapeDtypeStruct(A_x.shape, A_x.dtype),
        in_specs=[hbm] * 11,
        out_specs=pl.BlockSpec(memory_space=pltpu.VMEM),
        scratch_shapes=scratch_shapes,
        compiler_params=pltpu.CompilerParams(
            vmem_limit_bytes=100 * 1024 * 1024,
            disable_semaphore_checks=True,
        ),
    )(A_x, A_k_cache, A_v_cache, A_wq, A_wo.T, B_w_in, B_w_sp, B_b_sp, B_w_out.T, c, w_mod)
```

```python
import functools

import jax
import jax.numpy as jnp
from jax import lax
import jax.experimental.pallas as pl
import jax.experimental.pallas.tpu as pltpu

_D = 448
_HQ, _HKV, _DH = 16, 8, 256
_F = 1792
_FH = _F // 2
_EPS = 1e-5
_WOUT_SPLITS = (0, 256, 384, _D)

_F32 = jnp.float32
_BF16 = jnp.bfloat16


def _layernorm(x):
    m = jnp.mean(x, axis=-1, keepdims=True)
    d = x - m
    v = jnp.mean(d * d, axis=-1, keepdims=True)
    return d / jnp.sqrt(v + _EPS)


def _mm_nn(a, b):
    return lax.dot_general(a, b, (((1,), (0,)), ((), ())), preferred_element_type=_F32)


def _mm_nt(a, b):
    return lax.dot_general(a, b, (((1,), (1,)), ((), ())), preferred_element_type=_F32)


def _mod_chunk(mod, i):
    start = i * _D
    tile0 = (start // 128) * 128
    shift = start - tile0
    if shift == 0:
        return mod[:, start:start + _D]
    slab = mod[:, tile0:tile0 + 512]
    return pltpu.roll(slab, 512 - shift, 1)[:, :_D]


def _kernel(x_hbm, k_hbm, v_hbm, wq_hbm, wot_hbm, win_hbm, wsp_hbm, bsp_hbm, woutt_hbm,
            c_hbm, wmod_hbm,
            o_ref,
            x_v, c_v, wsp_v, bsp_v, wmod_v, wq_v, wot_v, win_v, woutt_v, k_v, v_v, sems,
            *, sk, w):
    copies = {}

    def start_copy(name, src, dst):
        cp = pltpu.make_async_copy(src, dst, sems.at[len(copies)])
        cp.start()
        copies[name] = cp

    start_copy("c", c_hbm, c_v)
    start_copy("x", x_hbm, x_v)
    start_copy("wmod", wmod_hbm, wmod_v)
    start_copy("wq", wq_hbm, wq_v)
    start_copy("k", k_hbm.at[0, :, pl.ds(sk - w, w), :], k_v)
    start_copy("v", v_hbm.at[0, :, pl.ds(sk - w, w), :], v_v)
    start_copy("wo", wot_hbm, wot_v)
    start_copy("win", win_hbm, win_v)
    n_wout = len(_WOUT_SPLITS) - 1
    for j in range(n_wout):
        a, b = _WOUT_SPLITS[j], _WOUT_SPLITS[j + 1]
        start_copy(f"wout{j}", woutt_hbm.at[pl.ds(a, b - a), :], woutt_v.at[pl.ds(a, b - a), :])
    start_copy("wsp", wsp_hbm, wsp_v)
    start_copy("bsp", bsp_hbm, bsp_v)

    copies["c"].wait()
    c = c_v[...].astype(_F32)
    silu_c = c * (1.0 / (1.0 + jnp.exp(-c)))
    silu_c = jnp.broadcast_to(silu_c, (8, _D)).astype(_BF16)
    copies["wsp"].wait()
    copies["bsp"].wait()
    w_sp = wsp_v[...].astype(_F32)
    b_sp = bsp_v[...].astype(_F32).reshape(1, 1)
    copies["x"].wait()
    x = jnp.broadcast_to(x_v[0].astype(_F32), (8, _D))
    xn = _layernorm(x)
    copies["wmod"].wait()
    mod = _mm_nn(silu_c, wmod_v[...])
    sa, ca, ga, sb, cb, gb = [_mod_chunk(mod, i) for i in range(6)]
    h1 = (xn * (1.0 + ca) + sa).astype(_BF16)

    copies["wq"].wait()
    row = lax.broadcasted_iota(jnp.int32, (8, _DH), 0)
    q = []
    for g in range(2):
        acc = jnp.zeros((8, _DH), _F32)
        for r in range(8):
            i = 8 * g + r
            qi = _mm_nn(h1, wq_v[:, i * _DH:(i + 1) * _DH])
            acc = jnp.where(row == r, qi, acc)
        q.append(acc.astype(_BF16))

    copies["k"].wait()
    row_w = lax.broadcasted_iota(jnp.int32, (8, w), 0)
    p, denom = [], []
    for g in range(2):
        s = jnp.zeros((8, w), _F32)
        for j in range(4):
            sj = _mm_nt(q[g], k_v[4 * g + j])
            s = jnp.where((row_w // 2) == j, sj, s)
        s = s * (_DH ** -0.5)
        m = jnp.max(s, axis=-1, keepdims=True)
        e = jnp.exp(s - m)
        denom.append(jnp.sum(e, axis=-1, keepdims=True))
        p.append(e.astype(_BF16))

    copies["v"].wait()
    o = []
    for g in range(2):
        acc = jnp.zeros((8, _DH), _F32)
        for j in range(4):
            oj = _mm_nn(p[g], v_v[4 * g + j])
            acc = jnp.where((row // 2) == j, oj, acc)
        o.append(acc / denom[g])

    copies["wo"].wait()
    att = jnp.zeros((8, _D), _F32)
    for i in range(_HQ):
        oi = jnp.where(row == (i % 8), o[i // 8], 0.0).astype(_BF16)
        att = att + _mm_nt(oi, wot_v[:, i * _DH:(i + 1) * _DH])
    att = jnp.broadcast_to(jnp.sum(att, axis=0, keepdims=True), (8, _D))
    x2 = x + ga * att
    h2 = (_layernorm(x2) * (1.0 + cb) + sb).astype(_BF16)

    copies["win"].wait()
    z2 = jax.nn.gelu(_mm_nn(h2, win_v[:, _FH:]), approximate=True)
    z2 = _layernorm(z2)
    z1 = jax.nn.gelu(_mm_nn(h2, win_v[:, :_FH]), approximate=True)
    u = (z1 * (w_sp * z2 + b_sp)).astype(_BF16)

    outs = []
    for j in range(n_wout):
        a, b = _WOUT_SPLITS[j], _WOUT_SPLITS[j + 1]
        copies[f"wout{j}"].wait()
        y = _mm_nt(u, woutt_v[a:b, :])
        outs.append(x2[:, a:b] + gb[:, a:b] * y)
    out = jnp.concatenate(outs, axis=1)
    o_ref[0] = out[0:1].astype(o_ref.dtype)


@jax.jit
def pallas_adaLN_cond__sliding_block_cached__mixer_gmlp__decode_kernel(
    A_x: jax.Array,
    A_k_cache: jax.Array,
    A_v_cache: jax.Array,
    A_wq: jax.Array,
    A_wo: jax.Array,
    B_x: jax.Array,
    B_w_in: jax.Array,
    B_w_sp: jax.Array,
    B_b_sp: jax.Array,
    B_w_out: jax.Array,
    c: jax.Array,
    w_mod: jax.Array,
):
    del B_x
    assert A_x.shape == (1, 1, _D) and c.shape == (1, _D)
    assert A_k_cache.shape == A_v_cache.shape
    assert (A_k_cache.shape[0], A_k_cache.shape[1], A_k_cache.shape[3]) == (1, _HKV, _DH)
    assert A_wq.shape == (_D, _HQ * _DH) and A_wo.shape == (_HQ * _DH, _D)
    assert B_w_in.shape == (_D, _F) and B_w_out.shape == (_FH, _D)
    assert B_w_sp.shape == (1, 1) and B_b_sp.shape == (1,) and w_mod.shape == (_D, 6 * _D)
    sk = A_k_cache.shape[2]
    w = min(4096, max(256, sk // 4))

    hbm = pl.BlockSpec(memory_space=pltpu.HBM)
    n_copies = 10 + len(_WOUT_SPLITS) - 1
    scratch_shapes = [
        pltpu.VMEM((1, 1, _D), _BF16),
        pltpu.VMEM((1, _D), _BF16),
        pltpu.VMEM((1, 1), _BF16),
        pltpu.VMEM((1,), _BF16),
        pltpu.VMEM((_D, 6 * _D), _BF16),
        pltpu.VMEM((_D, _HQ * _DH), _BF16),
        pltpu.VMEM((_D, _HQ * _DH), _BF16),
        pltpu.VMEM((_D, _F), _BF16),
        pltpu.VMEM((_D, _FH), _BF16),
        pltpu.VMEM((_HKV, w, _DH), _BF16),
        pltpu.VMEM((_HKV, w, _DH), _BF16),
        pltpu.SemaphoreType.DMA((n_copies,)),
    ]
    return pl.pallas_call(
        functools.partial(_kernel, sk=sk, w=w),
        out_shape=jax.ShapeDtypeStruct(A_x.shape, A_x.dtype),
        in_specs=[hbm] * 11,
        out_specs=pl.BlockSpec(memory_space=pltpu.VMEM),
        scratch_shapes=scratch_shapes,
        compiler_params=pltpu.CompilerParams(
            vmem_limit_bytes=100 * 1024 * 1024,
            disable_semaphore_checks=True,
        ),
    )(A_x, A_k_cache, A_v_cache, A_wq, A_wo.T, B_w_in, B_w_sp, B_b_sp, B_w_out.T, c, w_mod)
```

```python
import functools

import jax
import jax.numpy as jnp
from jax import lax
import jax.experimental.pallas as pl
import jax.experimental.pallas.tpu as pltpu

_D = 448
_HQ, _HKV, _DH = 16, 8, 256
_F = 1792
_FH = _F // 2
_EPS = 1e-5
_WOUT_SLABS = ((384, _D), (0, 256), (256, 384))

_F32 = jnp.float32
_BF16 = jnp.bfloat16


def _layernorm(x):
    m = jnp.mean(x, axis=-1, keepdims=True)
    d = x - m
    v = jnp.mean(d * d, axis=-1, keepdims=True)
    return d / jnp.sqrt(v + _EPS)


def _mm_nn(a, b):
    return lax.dot_general(a, b, (((1,), (0,)), ((), ())), preferred_element_type=_F32)


def _mm_nt(a, b):
    return lax.dot_general(a, b, (((1,), (1,)), ((), ())), preferred_element_type=_F32)


def _mod_chunk(mod, i):
    start = i * _D
    tile0 = (start // 128) * 128
    shift = start - tile0
    if shift == 0:
        return mod[:, start:start + _D]
    slab = mod[:, tile0:tile0 + 512]
    return pltpu.roll(slab, 512 - shift, 1)[:, :_D]


def _kernel(x_hbm, k_hbm, v_hbm, wq_hbm, wot_hbm, win_hbm, wsp_hbm, bsp_hbm, woutt_hbm,
            c_hbm, wmod_hbm,
            o_ref,
            x_v, c_v, wsp_v, bsp_v, wmod_v, wq_v, wot_v, win_v, woutt_v, k_v, v_v, sems,
            *, sk, w):
    copies = {}

    def start_copy(name, src, dst):
        cp = pltpu.make_async_copy(src, dst, sems.at[len(copies)])
        cp.start()
        copies[name] = cp

    start_copy("c", c_hbm, c_v)
    start_copy("x", x_hbm, x_v)
    start_copy("wmod", wmod_hbm, wmod_v)
    start_copy("wq", wq_hbm, wq_v)
    start_copy("k", k_hbm.at[0, :, pl.ds(sk - w, w), :], k_v)
    start_copy("v", v_hbm.at[0, :, pl.ds(sk - w, w), :], v_v)
    start_copy("wo", wot_hbm, wot_v)
    start_copy("win", win_hbm, win_v)
    for j, (a, b) in enumerate(_WOUT_SLABS):
        start_copy(f"wout{j}", woutt_hbm.at[pl.ds(a, b - a), :], woutt_v.at[pl.ds(a, b - a), :])
    start_copy("wsp", wsp_hbm, wsp_v)
    start_copy("bsp", bsp_hbm, bsp_v)

    copies["c"].wait()
    c = c_v[...].astype(_F32)
    silu_c = c * (1.0 / (1.0 + jnp.exp(-c)))
    silu_c = jnp.broadcast_to(silu_c, (8, _D)).astype(_BF16)
    copies["wsp"].wait()
    copies["bsp"].wait()
    w_sp = wsp_v[...].astype(_F32)
    b_sp = bsp_v[...].astype(_F32).reshape(1, 1)
    copies["x"].wait()
    x = jnp.broadcast_to(x_v[0].astype(_F32), (8, _D))
    xn = _layernorm(x)
    copies["wmod"].wait()
    mod = _mm_nn(silu_c, wmod_v[...])
    sa, ca, ga, sb, cb, gb = [_mod_chunk(mod, i) for i in range(6)]
    h1 = (xn * (1.0 + ca) + sa).astype(_BF16)

    copies["wq"].wait()
    row = lax.broadcasted_iota(jnp.int32, (8, _DH), 0)
    q = []
    for g in range(2):
        acc = jnp.zeros((8, _DH), _F32)
        for r in range(8):
            i = 8 * g + r
            qi = _mm_nn(h1, wq_v[:, i * _DH:(i + 1) * _DH])
            acc = jnp.where(row == r, qi, acc)
        q.append(acc.astype(_BF16))

    copies["k"].wait()
    row_w = lax.broadcasted_iota(jnp.int32, (8, w), 0)
    p, denom = [], []
    for g in range(2):
        s = jnp.zeros((8, w), _F32)
        for j in range(4):
            sj = _mm_nt(q[g], k_v[4 * g + j])
            s = jnp.where((row_w // 2) == j, sj, s)
        s = s * (_DH ** -0.5)
        m = jnp.max(s, axis=-1, keepdims=True)
        e = jnp.exp(s - m)
        denom.append(jnp.sum(e, axis=-1, keepdims=True))
        p.append(e.astype(_BF16))

    copies["v"].wait()
    o = []
    for g in range(2):
        acc = jnp.zeros((8, _DH), _F32)
        for j in range(4):
            oj = _mm_nn(p[g], v_v[4 * g + j])
            acc = jnp.where((row // 2) == j, oj, acc)
        o.append(acc / denom[g])

    copies["wo"].wait()
    att = jnp.zeros((8, _D), _F32)
    for i in range(_HQ):
        oi = jnp.where(row == (i % 8), o[i // 8], 0.0).astype(_BF16)
        att = att + _mm_nt(oi, wot_v[:, i * _DH:(i + 1) * _DH])
    att = jnp.broadcast_to(jnp.sum(att, axis=0, keepdims=True), (8, _D))
    x2 = x + ga * att
    h2 = (_layernorm(x2) * (1.0 + cb) + sb).astype(_BF16)

    copies["win"].wait()
    z2 = jax.nn.gelu(_mm_nn(h2, win_v[:, _FH:]), approximate=True)
    z2 = _layernorm(z2)
    z1 = jax.nn.gelu(_mm_nn(h2, win_v[:, :_FH]), approximate=True)
    u = (z1 * (w_sp * z2 + b_sp)).astype(_BF16)

    outs = {}
    for j, (a, b) in enumerate(_WOUT_SLABS):
        copies[f"wout{j}"].wait()
        y = _mm_nt(u, woutt_v[a:b, :])
        outs[a] = x2[:, a:b] + gb[:, a:b] * y
    out = jnp.concatenate([outs[a] for a in sorted(outs)], axis=1)
    o_ref[0] = out[0:1].astype(o_ref.dtype)


@jax.jit
def pallas_adaLN_cond__sliding_block_cached__mixer_gmlp__decode_kernel(
    A_x: jax.Array,
    A_k_cache: jax.Array,
    A_v_cache: jax.Array,
    A_wq: jax.Array,
    A_wo: jax.Array,
    B_x: jax.Array,
    B_w_in: jax.Array,
    B_w_sp: jax.Array,
    B_b_sp: jax.Array,
    B_w_out: jax.Array,
    c: jax.Array,
    w_mod: jax.Array,
):
    del B_x
    assert A_x.shape == (1, 1, _D) and c.shape == (1, _D)
    assert A_k_cache.shape == A_v_cache.shape
    assert (A_k_cache.shape[0], A_k_cache.shape[1], A_k_cache.shape[3]) == (1, _HKV, _DH)
    assert A_wq.shape == (_D, _HQ * _DH) and A_wo.shape == (_HQ * _DH, _D)
    assert B_w_in.shape == (_D, _F) and B_w_out.shape == (_FH, _D)
    assert B_w_sp.shape == (1, 1) and B_b_sp.shape == (1,) and w_mod.shape == (_D, 6 * _D)
    sk = A_k_cache.shape[2]
    w = min(4096, max(256, sk // 4))

    hbm = pl.BlockSpec(memory_space=pltpu.HBM)
    n_copies = 10 + len(_WOUT_SLABS)
    scratch_shapes = [
        pltpu.VMEM((1, 1, _D), _BF16),
        pltpu.VMEM((1, _D), _BF16),
        pltpu.VMEM((1, 1), _BF16),
        pltpu.VMEM((1,), _BF16),
        pltpu.VMEM((_D, 6 * _D), _BF16),
        pltpu.VMEM((_D, _HQ * _DH), _BF16),
        pltpu.VMEM((_D, _HQ * _DH), _BF16),
        pltpu.VMEM((_D, _F), _BF16),
        pltpu.VMEM((_D, _FH), _BF16),
        pltpu.VMEM((_HKV, w, _DH), _BF16),
        pltpu.VMEM((_HKV, w, _DH), _BF16),
        pltpu.SemaphoreType.DMA((n_copies,)),
    ]
    return pl.pallas_call(
        functools.partial(_kernel, sk=sk, w=w),
        out_shape=jax.ShapeDtypeStruct(A_x.shape, A_x.dtype),
        in_specs=[hbm] * 11,
        out_specs=pl.BlockSpec(memory_space=pltpu.VMEM),
        scratch_shapes=scratch_shapes,
        compiler_params=pltpu.CompilerParams(
            vmem_limit_bytes=64 * 1024 * 1024,
            disable_semaphore_checks=True,
        ),
    )(A_x, A_k_cache, A_v_cache, A_wq, A_wo.T, B_w_in, B_w_sp, B_b_sp, B_w_out.T, c, w_mod)
```
